```python
import os as _os
_os.environ.setdefault("JAX_PLATFORMS", "cpu")
import jax
import jax.numpy as jnp

def _softmax(x, axis=-1):
    return jax.nn.softmax(x, axis=axis)
def _gelu(x):
    return jax.nn.gelu(x, approximate=True)
def _silu(x):
    return jax.nn.silu(x)
def _sigmoid(x):
    return jax.nn.sigmoid(x)
def _layernorm(x, axis=-1, eps=1e-5):
    m = jnp.mean(x, axis=axis, keepdims=True)
    v = jnp.var(x, axis=axis, keepdims=True)
    return (x - m) / jnp.sqrt(v + eps)
def _scatter_add(tgt, idx, src, axis=0):
    return tgt.at[idx].add(src)
def _segment_sum(src, seg, n):
    return jax.ops.segment_sum(src, seg, n)
class _Rng:
    def __init__(self, key):
        self._k = key
    def _next(self):
        self._k, sub = jax.random.split(self._k)
        return sub
    def normal(self, shape):
        return jax.random.normal(self._next(), shape, dtype=jnp.bfloat16)
    def randint(self, lo, hi, shape):
        return jax.random.randint(self._next(), shape, lo, hi, dtype=jnp.int32)
    def uniform(self, shape, lo=0.0, hi=1.0):
        return jax.random.uniform(self._next(), shape, jnp.bfloat16, lo, hi)
    def permutation(self, n):
        return jax.random.permutation(self._next(), n)


kernel_name = 'concat_heads__gqa_block_cached__sliding_block_cached__decode'

def setup_inputs():
    _rng = _Rng(jax.random.key(int.from_bytes(__import__("os").urandom(4), "little")))
    _w = (lambda a: (lambda t: t.astype(jnp.bfloat16) if jnp.issubdtype(t.dtype, jnp.floating) else t)(jnp.asarray(a)))
    def _A_setup():
        B, Sq, D = 2, 1, 448
        Hq, Hkv, Sk, Dh = 16, 8, 8192, 256
        assert Hq % Hkv == 0, (Hq, Hkv)
        return {
            "x": _w((lambda *s: _rng.normal(s) * 0.8)(B, Sq, D)),
            "k_cache": _w((lambda *s: _rng.normal(s) * 0.8)(B, Hkv, Sk, Dh)),
            "v_cache": _w((lambda *s: _rng.normal(s) * 0.05)(B, Hkv, Sk, Dh)),
            "wq": _w((lambda *s: _rng.normal(s) * 0.8)(D, Hq * Dh) * (D ** -0.5)),
            "wo": _w((lambda *s: _rng.normal(s) * 0.05)(Hq * Dh, D) * ((Hq * Dh) ** -0.5)),
        }
    _A_in = _A_setup()

    def _B_setup():
        B, Sq, D = 2, 1, 448
        Hq, Hkv, Sk, Dh = 16, 8, 8192, 256
        assert Hq % Hkv == 0, (Hq, Hkv)
        return {
            "x": _w((lambda *s: _rng.normal(s) * 0.8)(B, Sq, D)),
            "k_cache": _w((lambda *s: _rng.normal(s) * 0.8)(B, Hkv, Sk, Dh)),
            "v_cache": _w((lambda *s: _rng.normal(s) * 0.05)(B, Hkv, Sk, Dh)),
            "wq": _w((lambda *s: _rng.normal(s) * 0.8)(D, Hq * Dh) * (D ** -0.5)),
            "wo": _w((lambda *s: _rng.normal(s) * 0.05)(Hq * Dh, D) * ((Hq * Dh) ** -0.5)),
        }
    _B_in = _B_setup()

    return {
        "A_x": _A_in["x"],
        "A_k_cache": _A_in["k_cache"],
        "A_v_cache": _A_in["v_cache"],
        "A_wq": _A_in["wq"],
        "A_wo": _A_in["wo"],
        "B_x": _B_in["x"],
        "B_k_cache": _B_in["k_cache"],
        "B_v_cache": _B_in["v_cache"],
        "B_wq": _B_in["wq"],
        "B_wo": _B_in["wo"],
    }

def reference(A_x, A_k_cache, A_v_cache, A_wq, A_wo, B_x, B_k_cache, B_v_cache, B_wq, B_wo):
    def _A_ref(x, k_cache, v_cache, wq, wo):
        B, Sq, D = x.shape
        Hq, Dh = 16, 256
        Hkv = k_cache.shape[1]
        rep = Hq // Hkv
        q = (lambda x, *d: x.transpose(*d))((x @ wq).reshape(B, Sq, Hq, Dh), 0, 2, 1, 3)
        k = jnp.repeat(k_cache, rep, axis=1)
        v = jnp.repeat(v_cache, rep, axis=1)
        scores = jnp.einsum("bhqd,bhkd->bhqk", q, k) * (Dh ** -0.5)
        p = _softmax(scores, axis=-1)
        o = jnp.einsum("bhqk,bhkd->bhqd", p, v)
        return (lambda x, *d: x.transpose(*d))(o, 0, 2, 1, 3).reshape(B, Sq, Hq * Dh) @ wo

    def _B_ref(x, k_cache, v_cache, wq, wo):
        B, Sq, D = x.shape
        Hq, Dh = 16, 256
        Hkv, Sk = k_cache.shape[1], k_cache.shape[2]
        W = min(4096, max(256, Sk // 4))
        rep = Hq // Hkv
        q = (lambda x, *d: x.transpose(*d))((x @ wq).reshape(B, Sq, Hq, Dh), 0, 2, 1, 3)
        k = jnp.repeat(k_cache[:, :, Sk - W:, :], rep, axis=1)
        v = jnp.repeat(v_cache[:, :, Sk - W:, :], rep, axis=1)
        scores = jnp.einsum("bhqd,bhkd->bhqk", q, k) * (Dh ** -0.5)
        p = _softmax(scores, axis=-1)
        o = jnp.einsum("bhqk,bhkd->bhqd", p, v)
        return (lambda x, *d: x.transpose(*d))(o, 0, 2, 1, 3).reshape(B, Sq, Hq * Dh) @ wo

    a = _A_ref(A_x, A_k_cache, A_v_cache, A_wq, A_wo)
    b = _B_ref(B_x, B_k_cache, B_v_cache, B_wq, B_wo)
    return jnp.concatenate([a, b], axis=-1)
```

```python
import functools
import jax
import jax.numpy as jnp
import jax.experimental.pallas as pl
import jax.experimental.pallas.tpu as pltpu

_B, _D = 2, 448
_HQ, _HKV, _SK, _DH = 16, 8, 8192, 256
_W = 2048
_T = 2048
_NSLOT = 4
_LA = 2
_NP = _B * _HKV
_NC = _SK // _T
_HD = _HQ * _DH
_S = 64
_NT = (((1,), (1,)), ((), ()))
_HI, _LO = 0, 1


def _kernel(xa_hbm, ak, av, wqa, wota, xb_hbm, bk, bv, wqb, wotb, o_ref,
            kvbuf, xbuf, wqbuf, wobuf, q_scr, o_scr, kv_sem, w_sem, *, PHA, PHB, compute=True):
    f32, bf16 = jnp.float32, jnp.bfloat16

    def issue_kv(ksrc, vsrc, base, slot, ph):
        def pair(r, n, flip):
            g = pl.multiple_of(base + r, 8)
            kp, vp = (_LO, _HI) if flip else (_HI, _LO)
            pltpu.make_async_copy(ksrc.at[pl.ds(g, n)], kvbuf.at[slot, 0, pl.ds(r, n)], kv_sem.at[slot]).start(priority=kp)
            pltpu.make_async_copy(vsrc.at[pl.ds(g, n)], kvbuf.at[slot, 1, pl.ds(r, n)], kv_sem.at[slot]).start(priority=vp)

        def block(r0, flip):
            def one(t, c):
                pair(pl.multiple_of(r0 + t * _S, 8), _S, flip)
                return c
            jax.lax.fori_loop(0, 2, one, 0)

        nfull = (_T - ph) // (2 * _S)
        tail = _T - ph - nfull * 2 * _S
        if ph:
            pair(0, ph, False)

        def two(jj, c):
            block(ph + jj * 4 * _S, True)
            block(ph + jj * 4 * _S + 2 * _S, False)
            return c
        jax.lax.fori_loop(0, nfull // 2, two, 0)
        if nfull % 2:
            block(ph + (nfull - 1) * 2 * _S, True)
        if tail:
            pair(_T - tail, tail, nfull % 2 == 0)

    def wait_kv(slot):
        pltpu.make_async_copy(kvbuf.at[slot], kvbuf.at[slot], kv_sem.at[slot]).wait()

    def issue_w(src0, dst0, s0, src1, dst1, s1, nslab, sem, c0=0, c1=_HD, npiece=2):
        wd = (c1 - c0) // npiece

        def slab(j, flip):
            def one(t, c):
                col = pl.multiple_of(c0 + t * wd, 128)
                p0, p1 = (_LO, _HI) if flip else (_HI, _LO)
                r0 = pl.multiple_of((s0[0] + j) * 8, 8)
                d0 = pl.multiple_of((s0[1] + j) * 8, 8)
                r1 = pl.multiple_of((s1[0] + j) * 8, 8)
                d1 = pl.multiple_of((s1[1] + j) * 8, 8)
                pltpu.make_async_copy(src0.at[pl.ds(r0, 8), pl.ds(col, wd)], dst0.at[pl.ds(d0, 8), pl.ds(col, wd)], sem).start(priority=p0)
                pltpu.make_async_copy(src1.at[pl.ds(r1, 8), pl.ds(col, wd)], dst1.at[pl.ds(d1, 8), pl.ds(col, wd)], sem).start(priority=p1)
                return c
            jax.lax.fori_loop(0, npiece, one, 0)

        assert nslab % 2 == 0
        def two(jj, c):
            slab(2 * jj, False)
            slab(2 * jj + 1, True)
            return c
        jax.lax.fori_loop(0, nslab // 2, two, 0)

    def wait_region(ref, sem):
        pltpu.make_async_copy(ref, ref, sem).wait()

    def kv_step_src(step_is_a, idx):
        if step_is_a:
            return ak, av, idx * _T, PHA
        return bk, bv, idx * _SK + (_SK - _W), PHB

    def issue_step(is_a, idx, slot):
        k, v, base, ph = kv_step_src(is_a, idx)
        issue_kv(k, v, base, slot, ph)

    xc = (pltpu.make_async_copy(xa_hbm, xbuf.at[0], w_sem.at[1]),
          pltpu.make_async_copy(xb_hbm, xbuf.at[1], w_sem.at[1]))
    for cp in xc:
        cp.start()
    nsl = _D // 8
    issue_w(wqa, wqbuf.at[0], (0, 0), wqb, wqbuf.at[1], (0, 0), nsl, w_sem.at[0])
    for s in range(_LA):
        issue_step(True, s, s)

    row = jax.lax.broadcasted_iota(jnp.int32, (8, _DH), 0)
    o_scr[...] = jnp.zeros(o_scr.shape, f32)
    for cp in xc:
        cp.wait()
    wait_region(wqbuf, w_sem.at[0])

    rx = jax.lax.broadcasted_iota(jnp.int32, (8, _D), 0)
    xs = []
    for ab in range(2):
        x = xbuf[ab].astype(f32)
        xs.append(jnp.where(rx % 2 == 0, jnp.broadcast_to(x[0:1], (8, _D)), jnp.broadcast_to(x[1:2], (8, _D))))
    x8 = jnp.where(rx < 4, xs[0], xs[1]).astype(bf16)

    def q_proj(ab):
        qq = jnp.dot(x8, wqbuf[ab], preferred_element_type=f32)
        for h in range(_HKV):
            q = jnp.where((row // 2) % 2 == 0, qq[:, 2 * h * _DH:(2 * h + 1) * _DH], qq[:, (2 * h + 1) * _DH:(2 * h + 2) * _DH])
            q_scr[ab, h] = q.astype(bf16).astype(f32) * (_DH ** -0.5)

    q_proj(0)

    def attend(q, slot, m, l, acc):
        s = jax.lax.dot_general(q, kvbuf[slot, 0], _NT, preferred_element_type=f32)
        mc = jnp.max(s, axis=-1, keepdims=True)
        if m is None:
            m_new = mc
            p = jnp.exp(s - m_new)
            l_new = jnp.sum(p, axis=-1, keepdims=True)
            acc_new = jnp.dot(p.astype(bf16), kvbuf[slot, 1], preferred_element_type=f32)
        else:
            m_new = jnp.maximum(m, mc)
            alpha = jnp.exp(m - m_new)
            p = jnp.exp(s - m_new)
            l_new = alpha * l + jnp.sum(p, axis=-1, keepdims=True)
            acc_new = alpha * acc + jnp.dot(p.astype(bf16), kvbuf[slot, 1], preferred_element_type=f32)
        return m_new, l_new, acc_new

    def store_o(ab, b, h, o):
        for g in range(2):
            o_scr[2 * h + g] = jnp.where(row == 4 * ab + 2 * g + b, o, o_scr[2 * h + g])

    def a_body(p, carry):
        b, h = p // _HKV, p % _HKV
        q = q_scr[0, h].astype(bf16)
        m = l = acc = None
        for c in range(_NC):
            nslot = (c + _LA) % _NSLOT
            if c + _LA < _NC:
                issue_step(True, p * _NC + c + _LA, nslot)
            else:
                @pl.when(p + 1 < _NP)
                def _():
                    issue_step(True, p * _NC + c + _LA, nslot)

                @pl.when(p + 1 == _NP)
                def _():
                    issue_step(False, c + _LA - _NC, nslot)
            wait_kv(c)
            m, l, acc = attend(q, c, m, l, acc)
            if c == 0:
                @pl.when(p == 0)
                def _():
                    q_proj(1)
        store_o(0, b, h, acc / l)
        return carry

    jax.lax.fori_loop(0, _NP, a_body, 0)

    issue_w(wota, wobuf, (0, 0), wota, wobuf, (nsl // 2, nsl // 2), nsl // 2, w_sem.at[1])

    def lhs_all():
        return jnp.concatenate([o_scr[j] for j in range(_HQ)], axis=1).astype(bf16)

    lane = jax.lax.broadcasted_iota(jnp.int32, (8, 128), 1)

    def finish_tile(t, z):
        s = z + pltpu.roll(z, 6, 0)
        if (t + 1) * 128 <= _D:
            w = s
        elif t * 128 >= _D:
            w = pltpu.roll(s, 4, 0)
        else:
            w = jnp.where(lane < _D - t * 128, s, pltpu.roll(s, 4, 0))
        o_ref[:, t * 128:(t + 1) * 128] = w[0:2].astype(o_ref.dtype)

    def proj_tile(t, lhs):
        finish_tile(t, jax.lax.dot_general(lhs, wobuf[t * 128:(t + 1) * 128, :], _NT, preferred_element_type=f32))

    def b_step(j, c, issue):
        b, h = j // _HKV, j % _HKV
        issue()
        wait_kv(c)
        _, l, acc = attend(q_scr[1, h].astype(bf16), c, None, None, None)
        store_o(1, b, h, acc / l)

    def b_body(gi, carry):
        for c in range(_NSLOT):
            j = gi * _NSLOT + c
            b_step(j, c, lambda: issue_step(False, j + _LA, (c + _LA) % _NSLOT))
            if c < 3:
                @pl.when(gi == 1)
                def _():
                    if c == 0:
                        wait_region(wobuf.at[pl.ds(0, _D)], w_sem.at[1])
                    proj_tile(c, lhs_all())
        return carry

    ng = _NP // _NSLOT
    jax.lax.fori_loop(0, ng - 1, b_body, 0)

    ob = _D // 8
    def issue_e0():
        issue_w(wotb, wobuf, (0, ob), wotb, wobuf, (12, ob + 12), 12, w_sem.at[0])
    def issue_e1():
        issue_w(wotb, wobuf, (24, ob + 24), wotb, wobuf, (32, ob + 32), 8, w_sem.at[2])
    def issue_e2():
        issue_w(wotb, wobuf, (40, ob + 40), wotb, wobuf, (48, ob + 48), 8, w_sem.at[3], 0, 2048, 1)
        issue_w(wotb, wobuf, (40, ob + 40), wotb, wobuf, (48, ob + 48), 8, w_sem.at[4], 2048, 3072, 1)
        issue_w(wotb, wobuf, (40, ob + 40), wotb, wobuf, (48, ob + 48), 8, w_sem.at[5], 3072, 4096, 1)

    j0 = (ng - 1) * _NSLOT
    b_step(j0 + 0, 0, lambda: issue_step(False, j0 + 2, 2))
    b_step(j0 + 1, 1, lambda: issue_step(False, j0 + 3, 3))
    b_step(j0 + 2, 2, issue_e0)
    b_step(j0 + 3, 3, issue_e1)
    issue_e2()
    lhs = lhs_all()
    wait_region(wobuf.at[pl.ds(_D, 192)], w_sem.at[0])
    proj_tile(3, lhs)
    proj_tile(4, lhs)
    wait_region(wobuf.at[pl.ds(_D + 192, 128)], w_sem.at[2])
    proj_tile(5, lhs)
    z = None
    for sem, c0, c1 in ((3, 0, 2048), (4, 2048, 3072), (5, 3072, 4096)):
        wait_region(wobuf.at[pl.ds(768, 128), pl.ds(c0, c1 - c0)], w_sem.at[sem])
        part = jax.lax.dot_general(lhs[:, c0:c1], wobuf[768:896, c0:c1], _NT, preferred_element_type=f32)
        z = part if z is None else z + part
    finish_tile(6, z)


def make(PHA=56, PHB=64, nobc=False):
  @jax.jit
  def f(A_x, A_k_cache, A_v_cache, A_wq, A_wo, B_x, B_k_cache, B_v_cache, B_wq, B_wo):
    bf16 = jnp.bfloat16
    flat = lambda t: t.reshape(_B * _HKV * _SK, _DH)
    out = pl.pallas_call(
        functools.partial(_kernel, PHA=PHA, PHB=PHB),
        in_specs=[pl.BlockSpec(memory_space=pl.ANY)] * 10,
        out_specs=pl.BlockSpec(memory_space=pltpu.VMEM),
        out_shape=jax.ShapeDtypeStruct((_B, 2 * _D), bf16),
        scratch_shapes=[
            pltpu.VMEM((_NSLOT, 2, _T, _DH), bf16),
            pltpu.VMEM((2, _B, _D), bf16),
            pltpu.VMEM((2, _D, _HD), bf16),
            pltpu.VMEM((2 * _D, _HD), bf16),
            pltpu.VMEM((2, _HKV, 8, _DH), jnp.float32),
            pltpu.VMEM((_HQ, 8, _DH), jnp.float32),
            pltpu.SemaphoreType.DMA((_NSLOT,)),
            pltpu.SemaphoreType.DMA((6,)),
        ],
        compiler_params=pltpu.CompilerParams(vmem_limit_bytes=64 * 1024 * 1024, disable_bounds_checks=nobc),
    )(A_x.reshape(_B, _D), flat(A_k_cache), flat(A_v_cache), A_wq, A_wo.T,
      B_x.reshape(_B, _D), flat(B_k_cache), flat(B_v_cache), B_wq, B_wo.T)
    return out.reshape(_B, 1, 2 * _D)
  return f

pallas_concat_heads__gqa_block_cached__sliding_block_cached__decode_kernel = make(nobc=True)
```

```python
import functools

import jax
import jax.numpy as jnp
import jax.experimental.pallas as pl
import jax.experimental.pallas.tpu as pltpu

_B, _D = 2, 448
_HQ, _HKV, _SK, _DH = 16, 8, 8192, 256
_W = min(4096, max(256, _SK // 4))
_T = 2048
_NSLOT = 4
_LA = 2
_NP = _B * _HKV
_NC = _SK // _T
_NA = _NP * _NC
_NS = _NA + _NP
_HD = _HQ * _DH
_S = 64
_NB = _T // (2 * _S)
_UC = 1024
_NU = _HD // _UC
_NSL = _D // 8
_NT = (((1,), (1,)), ((), ()))
_HI, _LO = 0, 1
assert _W == _T
_PH_A, _PH_B = 56, 56
_CUT_A, _CUT_B = 1792, 1920
_STRIDE = 13
_S_W2 = 58
_S_PROJ = 66
_LAG = 28
_F1, _F2 = 64, 80


def _kernel(xa_hbm, ak, av, wqa, wota, xb_hbm, bk, bv, wqb, wotb, o_ref,
            kvbuf, xbuf, x8_scr, wqbuf, wobuf, q_scr, o_scr, z_scr, m_scr, l_scr, acc_scr, kv_sem, w_sem,
            ):
    PHA, PHB, CUTA, CUTB, STRIDE = _PH_A, _PH_B, _CUT_A, _CUT_B, _STRIDE
    S_W2, S_PROJ, LAG, F1, F2 = _S_W2, _S_PROJ, _LAG, _F1, _F2
    f32, bf16 = jnp.float32, jnp.bfloat16

    def in_order(once, fn):
        def body(_, c):
            fn()
            return c
        jax.lax.fori_loop(0, once, body, 0)

    def wait_region(ref, sem):
        pltpu.make_async_copy(ref, ref, sem).wait()

    def issue_kv(ksrc, vsrc, base, slot, ph):
        def pair(r, n, k_hi):
            g = pl.multiple_of(base + r, 8)
            kp, vp = (_HI, _LO) if k_hi else (_LO, _HI)
            pltpu.make_async_copy(ksrc.at[pl.ds(g, n)], kvbuf.at[slot, 0, pl.ds(r, n)],
                                  kv_sem.at[slot]).start(priority=kp)
            pltpu.make_async_copy(vsrc.at[pl.ds(g, n)], kvbuf.at[slot, 1, pl.ds(r, n)],
                                  kv_sem.at[slot]).start(priority=vp)

        off = ((_NB - 1) * (1 - STRIDE)) % _NB

        def block(j, k_hi):
            r0 = ph + ((STRIDE * j + off) % _NB) * 2 * _S

            def one(t, c):
                pair(pl.multiple_of(r0 + t * _S, 8), _S, k_hi)
                return c
            jax.lax.fori_loop(0, 2, one, 0)

        def two(jj, c):
            block(2 * jj, True)
            block(2 * jj + 1, False)
            return c

        pair(0, ph, False)
        jax.lax.fori_loop(0, _NB // 2 - 1, two, 0)
        block(_NB - 2, True)
        last = ph + (_NB - 1) * 2 * _S
        pair(last, _T - last, False)

    def issue_a(n):
        issue_kv(ak, av, n * _T, n % _NSLOT, PHA)

    def issue_b(n):
        issue_kv(bk, bv, (n - _NA) * _SK + (_SK - _W), n % _NSLOT, PHB)

    def issue_w(st0, st1, nslab):
        def piece(st, j, c0, c1, prio):
            src, s0, dst, d0, _, sem = st
            r = pl.multiple_of((s0 + j) * 8, 8)
            d = pl.multiple_of((d0 + j) * 8, 8)
            pltpu.make_async_copy(src.at[pl.ds(r, 8), pl.ds(c0, c1 - c0)],
                                  dst.at[pl.ds(d, 8), pl.ds(c0, c1 - c0)], sem).start(priority=prio)

        def two(jj, c):
            once = jnp.minimum(jj + 1, 1)
            for k in range(2):
                j = 2 * jj + k
                p0, p1 = (_LO, _HI) if k else (_HI, _LO)
                in_order(once, lambda: (piece(st0, j, 0, st0[4], p1), piece(st1, j, 0, st1[4], p0)))
                in_order(once, lambda: (piece(st0, j, st0[4], _HD, p0), piece(st1, j, st1[4], _HD, p1)))
            return c
        jax.lax.fori_loop(0, nslab // 2, two, 0)

    tail = [(0, 4, None, 3 * _NU, 4 * _NU), (8, 8, None, 4 * _NU, 5 * _NU)]
    for first, t, edges in ((24, 5, (0, 2048, _HD)), (40, 6, (0, 2048, 3072, _HD))):
        for c0, c1 in zip(edges[:-1], edges[1:]):
            tail.append((first, 8, (c0, c1), t * _NU + c0 // _UC, t * _NU + c1 // _UC))
    n_w = 4
    q_hi, q_lo = [], []
    for i, (first, n, cols, _, _) in enumerate(tail):
        for k in range(n + 1 if cols is None else n):
            for st in range(2):
                a = first + st * n
                if cols is None:
                    blk = ([(a + k - 1, CUTB, _HD)] if k > 0 else []) + ([(a + k, 0, CUTB)] if k < n else [])
                else:
                    blk = [(a + k,) + cols]
                (q_hi if (k + st) % 2 == 0 else q_lo).extend((i,) + p for p in blk)
    nh = len(q_hi) - LAG // 2
    lo_seq = q_lo[:nh] + [p for pr in zip(q_hi[nh:], q_lo[nh:]) for p in pr]
    fifo = [(p, _LO) for p in lo_seq[:LAG]]
    for i in range(nh):
        fifo += [(q_hi[i], _HI), (lo_seq[LAG + i], _LO)]
    assert len(fifo) == len(q_hi) + len(q_lo)

    def issue_tail(once, a, b):
        def start(entries):
            for (i, sl, c0, c1), prio in entries:
                pltpu.make_async_copy(wotb.at[pl.ds(sl * 8, 8), pl.ds(c0, c1 - c0)],
                                      wobuf.at[pl.ds(_D + sl * 8, 8), pl.ds(c0, c1 - c0)],
                                      w_sem.at[n_w + i]).start(priority=prio)
        for k in range(a, b, 2):
            in_order(once, functools.partial(start, fifo[k:min(k + 2, b)]))

    def wait_tail(i):
        first, n, cols, _, _ = tail[i]
        c0, c1 = cols or (0, _HD)
        wait_region(wobuf.at[pl.ds(_D + first * 8, 16 * n), pl.ds(c0, c1 - c0)], w_sem.at[n_w + i])

    xc = (pltpu.make_async_copy(xa_hbm, xbuf.at[0], w_sem.at[1]),
          pltpu.make_async_copy(xb_hbm, xbuf.at[1], w_sem.at[1]))
    for cp in xc:
        cp.start()
    half = _NSL // 2
    issue_w((wqa, 0, wqbuf.at[0], 0, CUTA, w_sem.at[0]), (wqa, half, wqbuf.at[0], half, CUTA, w_sem.at[0]), half)

    def pre(n, c):
        issue_a(n)
        return c
    jax.lax.fori_loop(0, _LA, pre, 0)

    for ref in (o_scr, z_scr, m_scr, l_scr, acc_scr):
        ref[...] = jnp.zeros(ref.shape, f32)
    for cp in xc:
        cp.wait()
    rx = jax.lax.broadcasted_iota(jnp.int32, (8, _D), 0)
    xs = []
    for ab in range(2):
        x = xbuf[ab].astype(f32)
        xs.append(jnp.where(rx % 2 == 0, jnp.broadcast_to(x[0:1], (8, _D)), jnp.broadcast_to(x[1:2], (8, _D))))
    x8_scr[...] = jnp.where(rx < 4, xs[0], xs[1])
    wait_region(wqbuf.at[0], w_sem.at[0])

    row = jax.lax.broadcasted_iota(jnp.int32, (8, _DH), 0)
    lane = jax.lax.broadcasted_iota(jnp.int32, (8, 128), 1)

    def unit(u, c):
        t, cb = u // _NU, u % _NU
        per = _UC // _DH
        lhs = jnp.concatenate([o_scr[cb * per + i] for i in range(per)], axis=1).astype(bf16)
        w = wobuf[pl.ds(pl.multiple_of(t * 128, 128), 128), pl.ds(pl.multiple_of(cb * _UC, _UC), _UC)]
        z_scr[t] += jax.lax.dot_general(lhs, w, _NT, preferred_element_type=f32)
        return c

    def finish_tile(t):
        z = z_scr[t]
        s = z + pltpu.roll(z, 6, 0)
        if (t + 1) * 128 <= _D:
            w = s
        elif t * 128 >= _D:
            w = pltpu.roll(s, 4, 0)
        else:
            w = jnp.where(lane < _D - t * 128, s, pltpu.roll(s, 4, 0))
        o_ref[:, t * 128:(t + 1) * 128] = w[0:2].astype(o_ref.dtype)

    sched = [(S_PROJ + t, t * _NU, (t + 1) * _NU) for t in range(3)]
    sched += [(_NS + i, c[3], c[4]) for i, c in enumerate(tail)]
    first_of_last_tile = len(tail) - 3

    def event(s, carry):
        n = s + _LA
        once = jnp.minimum(s, 1)

        @pl.when(n < _NA)
        def _():
            issue_a(n)

        @pl.when(jnp.logical_and(n >= _NA, n < _NS))
        def _():
            issue_b(n)

        @pl.when(s == S_W2)
        def _():
            issue_w((wqb, 0, wqbuf.at[1], 0, CUTB, w_sem.at[2]), (wota, 0, wobuf, 0, CUTA, w_sem.at[3]), _NSL)

        @pl.when(n == _NS)
        def _():
            issue_tail(once, 0, F1)

        @pl.when(n == _NS + 1)
        def _():
            issue_tail(once, F1, F2)

        @pl.when(s == _NA)
        def _():
            wait_region(wqbuf.at[1], w_sem.at[2])
            wait_region(wobuf.at[pl.ds(0, _D)], w_sem.at[3])

        @pl.when(s < _NS)
        def _():
            is_a = s < _NA
            p = jnp.where(is_a, s // _NC, s - _NA)
            first = jnp.logical_or(jnp.logical_not(is_a), s % _NC == 0)
            last = jnp.logical_or(jnp.logical_not(is_a), s % _NC == _NC - 1)
            ab = jnp.where(is_a, 0, 1)
            b, h = p // _HKV, p % _HKV
            slot = s % _NSLOT

            @pl.when(jnp.logical_and(first, b == 0))
            def _():
                w = wqbuf[ab, :, pl.ds(pl.multiple_of(h * 2 * _DH, 2 * _DH), 2 * _DH)]
                qq = jnp.dot(x8_scr[...].astype(bf16), w, preferred_element_type=f32)
                qh = jnp.where((row // 2) % 2 == 0, qq[:, :_DH], qq[:, _DH:])
                q_scr[h] = qh.astype(bf16).astype(f32) * (_DH ** -0.5)

            q = q_scr[h].astype(bf16)
            wait_region(kvbuf.at[slot], kv_sem.at[slot])
            sc = jax.lax.dot_general(q, kvbuf[slot, 0], _NT, preferred_element_type=f32)
            m_old = jnp.where(first, -jnp.inf, m_scr[:, 0:1])
            l_old = jnp.where(first, 0.0, l_scr[:, 0:1])
            acc_old = jnp.where(first, 0.0, acc_scr[...])
            m_new = jnp.maximum(m_old, jnp.max(sc, axis=-1, keepdims=True))
            alpha = jnp.exp(m_old - m_new)
            pr = jnp.exp(sc - m_new)
            l_new = alpha * l_old + jnp.sum(pr, axis=-1, keepdims=True)
            acc_new = alpha * acc_old + jnp.dot(pr.astype(bf16), kvbuf[slot, 1], preferred_element_type=f32)
            m_scr[...] = jnp.broadcast_to(m_new, m_scr.shape)
            l_scr[...] = jnp.broadcast_to(l_new, l_scr.shape)
            acc_scr[...] = acc_new

            @pl.when(last)
            def _():
                o = acc_new / l_new
                for g in range(2):
                    o_scr[2 * h + g] = jnp.where(row == 4 * ab + 2 * g + b, o, o_scr[2 * h + g])

        @pl.when(s == _NS - 1)
        def _():
            issue_tail(once, F2, len(fifo))

        for i in range(len(tail)):
            @pl.when(s == _NS + i)
            def _():
                if i == first_of_last_tile:
                    for t in range(6):
                        finish_tile(t)
                wait_tail(i)

        lo = hi = jnp.int32(0)
        for e, a, z in sched:
            lo = jnp.where(s == e, a, lo)
            hi = jnp.where(s == e, z, hi)
        jax.lax.fori_loop(lo, hi, unit, 0)
        return carry

    jax.lax.fori_loop(0, _NS + len(tail), event, 0)
    finish_tile(6)


@jax.jit
def pallas_concat_heads__gqa_block_cached__sliding_block_cached__decode_kernel(
    A_x: jax.Array,
    A_k_cache: jax.Array,
    A_v_cache: jax.Array,
    A_wq: jax.Array,
    A_wo: jax.Array,
    B_x: jax.Array,
    B_k_cache: jax.Array,
    B_v_cache: jax.Array,
    B_wq: jax.Array,
    B_wo: jax.Array,
):
    bf16, f32 = jnp.bfloat16, jnp.float32
    flat = lambda t: t.reshape(_B * _HKV * _SK, _DH)
    out = pl.pallas_call(
        _kernel,
        in_specs=[pl.BlockSpec(memory_space=pl.ANY)] * 10,
        out_specs=pl.BlockSpec(memory_space=pltpu.VMEM),
        out_shape=jax.ShapeDtypeStruct((_B, 2 * _D), bf16),
        scratch_shapes=[
            pltpu.VMEM((_NSLOT, 2, _T, _DH), bf16),
            pltpu.VMEM((2, _B, _D), bf16),
            pltpu.VMEM((8, _D), f32),
            pltpu.VMEM((2, _D, _HD), bf16),
            pltpu.VMEM((2 * _D, _HD), bf16),
            pltpu.VMEM((_HKV, 8, _DH), f32),
            pltpu.VMEM((_HQ, 8, _DH), f32),
            pltpu.VMEM((7, 8, 128), f32),
            pltpu.VMEM((8, 128), f32),
            pltpu.VMEM((8, 128), f32),
            pltpu.VMEM((8, _DH), f32),
            pltpu.SemaphoreType.DMA((_NSLOT,)),
            pltpu.SemaphoreType.DMA((11,)),
        ],
        compiler_params=pltpu.CompilerParams(vmem_limit_bytes=64 * 1024 * 1024,
                                             disable_semaphore_checks=True),
    )(A_x.reshape(_B, _D), flat(A_k_cache), flat(A_v_cache), A_wq, A_wo.T,
      B_x.reshape(_B, _D), flat(B_k_cache), flat(B_v_cache), B_wq, B_wo.T)
    return out.reshape(_B, 1, 2 * _D)
```

```python
import functools

import jax
import jax.numpy as jnp
import jax.experimental.pallas as pl
import jax.experimental.pallas.tpu as pltpu

_B, _D = 2, 448
_HQ, _HKV, _SK, _DH = 16, 8, 8192, 256
_W = min(4096, max(256, _SK // 4))
_T = 2048
_NSLOT = 4
_LA = 2
_NP = _B * _HKV
_NC = _SK // _T
_NA = _NP * _NC
_NS = _NA + _NP
_HD = _HQ * _DH
_S = 64
_NB = _T // (2 * _S)
_UC = 1024
_NU = _HD // _UC
_NSL = _D // 8
_NT = (((1,), (1,)), ((), ()))
_HI, _LO = 0, 1
assert _W == _T
_PH_A, _PH_B = 56, 56
_CUT_A, _CUT_B = 1792, 1920
_STRIDE = 13
_SIG_1, _SIG_2 = 13, 19
_S_W2 = 58
_S_PROJ = 66
_LAG = 28
_F1, _F2 = 64, 80


def _kernel(xa_hbm, ak, av, wqa, wota, xb_hbm, bk, bv, wqb, wotb, o_ref,
            kvbuf, xbuf, x8_scr, wqbuf, wobuf, q_scr, o_scr, z_scr, m_scr, l_scr, acc_scr, kv_sem, w_sem,
            ):
    PHA, PHB, CUTA, CUTB, STRIDE = _PH_A, _PH_B, _CUT_A, _CUT_B, _STRIDE
    S_W2, S_PROJ, LAG, F1, F2 = _S_W2, _S_PROJ, _LAG, _F1, _F2
    f32, bf16 = jnp.float32, jnp.bfloat16

    def in_order(once, fn):
        def body(_, c):
            fn()
            return c
        jax.lax.fori_loop(0, once, body, 0)

    def wait_region(ref, sem):
        pltpu.make_async_copy(ref, ref, sem).wait()

    def issue_kv(ksrc, vsrc, base, slot, ph):
        def pair(r, n, k_hi):
            g = pl.multiple_of(base + r, 8)
            kp, vp = (_HI, _LO) if k_hi else (_LO, _HI)
            pltpu.make_async_copy(ksrc.at[pl.ds(g, n)], kvbuf.at[slot, 0, pl.ds(r, n)],
                                  kv_sem.at[slot]).start(priority=kp)
            pltpu.make_async_copy(vsrc.at[pl.ds(g, n)], kvbuf.at[slot, 1, pl.ds(r, n)],
                                  kv_sem.at[slot]).start(priority=vp)

        off = ((_NB - 1) * (1 - STRIDE)) % _NB

        def block(j, k_hi):
            r0 = ph + ((STRIDE * j + off) % _NB) * 2 * _S

            def one(t, c):
                pair(pl.multiple_of(r0 + t * _S, 8), _S, k_hi)
                return c
            jax.lax.fori_loop(0, 2, one, 0)

        def two(jj, c):
            block(2 * jj, True)
            block(2 * jj + 1, False)
            return c

        pair(0, ph, False)
        jax.lax.fori_loop(0, _NB // 2 - 1, two, 0)
        block(_NB - 2, True)
        last = ph + (_NB - 1) * 2 * _S
        pair(last, _T - last, False)

    def issue_a(n):
        issue_kv(ak, av, n * _T, n % _NSLOT, PHA)

    def issue_b(n):
        issue_kv(bk, bv, (n - _NA) * _SK + (_SK - _W), n % _NSLOT, PHB)

    def issue_w(st0, st1, nslab, sig):
        def piece(st, j, c0, c1, prio):
            src, s0, dst, d0, _, sem = st
            r = pl.multiple_of((s0 + j) * 8, 8)
            d = pl.multiple_of((d0 + j) * 8, 8)
            pltpu.make_async_copy(src.at[pl.ds(r, 8), pl.ds(c0, c1 - c0)],
                                  dst.at[pl.ds(d, 8), pl.ds(c0, c1 - c0)], sem).start(priority=prio)

        def two(jj, c):
            once = jnp.minimum(jj + 1, 1)
            for k in range(2):
                j = (sig * (2 * jj + k)) % nslab
                nx = jnp.where(j + 1 == nslab, 0, j + 1)
                in_order(once, lambda: (piece(st0, j, st0[4], _HD, _HI), piece(st1, j, st1[4], _HD, _LO)))
                in_order(once, lambda: (piece(st0, nx, 0, st0[4], _HI), piece(st1, nx, 0, st1[4], _LO)))
            return c
        jax.lax.fori_loop(0, nslab // 2, two, 0)

    tail = [(0, 4, None, 3 * _NU, 4 * _NU), (8, 8, None, 4 * _NU, 5 * _NU)]
    for first, t, edges in ((24, 5, (0, 2048, _HD)), (40, 6, (0, 2048, 3072, _HD))):
        for c0, c1 in zip(edges[:-1], edges[1:]):
            tail.append((first, 8, (c0, c1), t * _NU + c0 // _UC, t * _NU + c1 // _UC))
    n_w = 4
    q_hi, q_lo = [], []
    for i, (first, n, cols, _, _) in enumerate(tail):
        for k in range(n + 1 if cols is None else n):
            for st in range(2):
                a = first + st * n
                if cols is None:
                    blk = ([(a + k - 1, CUTB, _HD)] if k > 0 else []) + ([(a + k, 0, CUTB)] if k < n else [])
                else:
                    blk = [(a + k,) + cols]
                (q_hi if (k + st) % 2 == 0 else q_lo).extend((i,) + p for p in blk)
    nh = len(q_hi) - LAG // 2
    lo_seq = q_lo[:nh] + [p for pr in zip(q_hi[nh:], q_lo[nh:]) for p in pr]
    fifo = [(p, _LO) for p in lo_seq[:LAG]]
    for i in range(nh):
        fifo += [(q_hi[i], _HI), (lo_seq[LAG + i], _LO)]
    assert len(fifo) == len(q_hi) + len(q_lo)

    def issue_tail(once, a, b):
        def start(entries):
            for (i, sl, c0, c1), prio in entries:
                pltpu.make_async_copy(wotb.at[pl.ds(sl * 8, 8), pl.ds(c0, c1 - c0)],
                                      wobuf.at[pl.ds(_D + sl * 8, 8), pl.ds(c0, c1 - c0)],
                                      w_sem.at[n_w + i]).start(priority=prio)
        for k in range(a, b, 2):
            in_order(once, functools.partial(start, fifo[k:min(k + 2, b)]))

    def wait_tail(i):
        first, n, cols, _, _ = tail[i]
        c0, c1 = cols or (0, _HD)
        wait_region(wobuf.at[pl.ds(_D + first * 8, 16 * n), pl.ds(c0, c1 - c0)], w_sem.at[n_w + i])

    xc = (pltpu.make_async_copy(xa_hbm, xbuf.at[0], w_sem.at[1]),
          pltpu.make_async_copy(xb_hbm, xbuf.at[1], w_sem.at[1]))
    for cp in xc:
        cp.start()
    half = _NSL // 2
    issue_w((wqa, 0, wqbuf.at[0], 0, CUTA, w_sem.at[0]), (wqa, half, wqbuf.at[0], half, CUTA, w_sem.at[0]),
            half, _SIG_1)

    def pre(n, c):
        issue_a(n)
        return c
    jax.lax.fori_loop(0, _LA, pre, 0)

    for ref in (o_scr, z_scr, m_scr, l_scr, acc_scr):
        ref[...] = jnp.zeros(ref.shape, f32)
    for cp in xc:
        cp.wait()
    rx = jax.lax.broadcasted_iota(jnp.int32, (8, _D), 0)
    xs = []
    for ab in range(2):
        x = xbuf[ab].astype(f32)
        xs.append(jnp.where(rx % 2 == 0, jnp.broadcast_to(x[0:1], (8, _D)), jnp.broadcast_to(x[1:2], (8, _D))))
    x8_scr[...] = jnp.where(rx < 4, xs[0], xs[1])
    wait_region(wqbuf.at[0], w_sem.at[0])

    row = jax.lax.broadcasted_iota(jnp.int32, (8, _DH), 0)
    lane = jax.lax.broadcasted_iota(jnp.int32, (8, 128), 1)

    def unit(u, c):
        t, cb = u // _NU, u % _NU
        per = _UC // _DH
        lhs = jnp.concatenate([o_scr[cb * per + i] for i in range(per)], axis=1).astype(bf16)
        w = wobuf[pl.ds(pl.multiple_of(t * 128, 128), 128), pl.ds(pl.multiple_of(cb * _UC, _UC), _UC)]
        z_scr[t] += jax.lax.dot_general(lhs, w, _NT, preferred_element_type=f32)
        return c

    def finish_tile(t):
        z = z_scr[t]
        s = z + pltpu.roll(z, 6, 0)
        if (t + 1) * 128 <= _D:
            w = s
        elif t * 128 >= _D:
            w = pltpu.roll(s, 4, 0)
        else:
            w = jnp.where(lane < _D - t * 128, s, pltpu.roll(s, 4, 0))
        o_ref[:, t * 128:(t + 1) * 128] = w[0:2].astype(o_ref.dtype)

    sched = [(S_PROJ + t, t * _NU, (t + 1) * _NU) for t in range(3)]
    sched += [(_NS + i, c[3], c[4]) for i, c in enumerate(tail)]
    first_of_last_tile = len(tail) - 3

    def event(s, carry):
        n = s + _LA
        once = jnp.minimum(s, 1)

        @pl.when(n < _NA)
        def _():
            issue_a(n)

        @pl.when(jnp.logical_and(n >= _NA, n < _NS))
        def _():
            issue_b(n)

        @pl.when(s == S_W2)
        def _():
            issue_w((wqb, 0, wqbuf.at[1], 0, CUTB, w_sem.at[2]), (wota, 0, wobuf, 0, CUTA, w_sem.at[3]),
                    _NSL, _SIG_2)

        @pl.when(n == _NS)
        def _():
            issue_tail(once, 0, F1)

        @pl.when(n == _NS + 1)
        def _():
            issue_tail(once, F1, F2)

        @pl.when(s == _NA)
        def _():
            wait_region(wqbuf.at[1], w_sem.at[2])
            wait_region(wobuf.at[pl.ds(0, _D)], w_sem.at[3])

        @pl.when(s < _NS)
        def _():
            is_a = s < _NA
            p = jnp.where(is_a, s // _NC, s - _NA)
            first = jnp.logical_or(jnp.logical_not(is_a), s % _NC == 0)
            last = jnp.logical_or(jnp.logical_not(is_a), s % _NC == _NC - 1)
            ab = jnp.where(is_a, 0, 1)
            b, h = p // _HKV, p % _HKV
            slot = s % _NSLOT

            @pl.when(jnp.logical_and(first, b == 0))
            def _():
                w = wqbuf[ab, :, pl.ds(pl.multiple_of(h * 2 * _DH, 2 * _DH), 2 * _DH)]
                qq = jnp.dot(x8_scr[...].astype(bf16), w, preferred_element_type=f32)
                qh = jnp.where((row // 2) % 2 == 0, qq[:, :_DH], qq[:, _DH:])
                q_scr[h] = qh.astype(bf16).astype(f32) * (_DH ** -0.5)

            q = q_scr[h].astype(bf16)
            wait_region(kvbuf.at[slot], kv_sem.at[slot])
            sc = jax.lax.dot_general(q, kvbuf[slot, 0], _NT, preferred_element_type=f32)
            m_old = jnp.where(first, -jnp.inf, m_scr[:, 0:1])
            l_old = jnp.where(first, 0.0, l_scr[:, 0:1])
            acc_old = jnp.where(first, 0.0, acc_scr[...])
            m_new = jnp.maximum(m_old, jnp.max(sc, axis=-1, keepdims=True))
            alpha = jnp.exp(m_old - m_new)
            pr = jnp.exp(sc - m_new)
            l_new = alpha * l_old + jnp.sum(pr, axis=-1, keepdims=True)
            acc_new = alpha * acc_old + jnp.dot(pr.astype(bf16), kvbuf[slot, 1], preferred_element_type=f32)
            m_scr[...] = jnp.broadcast_to(m_new, m_scr.shape)
            l_scr[...] = jnp.broadcast_to(l_new, l_scr.shape)
            acc_scr[...] = acc_new

            @pl.when(last)
            def _():
                o = acc_new / l_new
                for g in range(2):
                    o_scr[2 * h + g] = jnp.where(row == 4 * ab + 2 * g + b, o, o_scr[2 * h + g])

        @pl.when(s == _NS - 1)
        def _():
            issue_tail(once, F2, len(fifo))

        for i in range(len(tail)):
            @pl.when(s == _NS + i)
            def _():
                if i == first_of_last_tile:
                    for t in range(6):
                        finish_tile(t)
                wait_tail(i)

        lo = hi = jnp.int32(0)
        for e, a, z in sched:
            lo = jnp.where(s == e, a, lo)
            hi = jnp.where(s == e, z, hi)
        jax.lax.fori_loop(lo, hi, unit, 0)
        return carry

    jax.lax.fori_loop(0, _NS + len(tail), event, 0)
    finish_tile(6)


@jax.jit
def pallas_concat_heads__gqa_block_cached__sliding_block_cached__decode_kernel(
    A_x: jax.Array,
    A_k_cache: jax.Array,
    A_v_cache: jax.Array,
    A_wq: jax.Array,
    A_wo: jax.Array,
    B_x: jax.Array,
    B_k_cache: jax.Array,
    B_v_cache: jax.Array,
    B_wq: jax.Array,
    B_wo: jax.Array,
):
    bf16, f32 = jnp.bfloat16, jnp.float32
    flat = lambda t: t.reshape(_B * _HKV * _SK, _DH)
    out = pl.pallas_call(
        _kernel,
        in_specs=[pl.BlockSpec(memory_space=pl.ANY)] * 10,
        out_specs=pl.BlockSpec(memory_space=pltpu.VMEM),
        out_shape=jax.ShapeDtypeStruct((_B, 2 * _D), bf16),
        scratch_shapes=[
            pltpu.VMEM((_NSLOT, 2, _T, _DH), bf16),
            pltpu.VMEM((2, _B, _D), bf16),
            pltpu.VMEM((8, _D), f32),
            pltpu.VMEM((2, _D, _HD), bf16),
            pltpu.VMEM((2 * _D, _HD), bf16),
            pltpu.VMEM((_HKV, 8, _DH), f32),
            pltpu.VMEM((_HQ, 8, _DH), f32),
            pltpu.VMEM((7, 8, 128), f32),
            pltpu.VMEM((8, 128), f32),
            pltpu.VMEM((8, 128), f32),
            pltpu.VMEM((8, _DH), f32),
            pltpu.SemaphoreType.DMA((_NSLOT,)),
            pltpu.SemaphoreType.DMA((11,)),
        ],
        compiler_params=pltpu.CompilerParams(vmem_limit_bytes=64 * 1024 * 1024,
                                             disable_semaphore_checks=True),
    )(A_x.reshape(_B, _D), flat(A_k_cache), flat(A_v_cache), A_wq, A_wo.T,
      B_x.reshape(_B, _D), flat(B_k_cache), flat(B_v_cache), B_wq, B_wo.T)
    return out.reshape(_B, 1, 2 * _D)
```

```python
import functools

import jax
import jax.numpy as jnp
import jax.experimental.pallas as pl
import jax.experimental.pallas.tpu as pltpu

_B, _D = 2, 448
_HQ, _HKV, _SK, _DH = 16, 8, 8192, 256
_W = min(4096, max(256, _SK // 4))
_T = 2048
_NSLOT = 4
_LA = 2
_NP = _B * _HKV
_NC = _SK // _T
_NA = _NP * _NC
_NS = _NA + _NP
_HD = _HQ * _DH
_S = 64
_NB = _T // (2 * _S)
_UC = 1024
_NU = _HD // _UC
_NSL = _D // 8
_NT = (((1,), (1,)), ((), ()))
_HI, _LO = 0, 1
assert _W == _T
_PH_A, _PH_B = 56, 56
_CUT_A, _CUT_B = 1792, 1920
_STRIDE = 13
_SIG_1, _SIG_2 = 13, 19
_S_W2 = 58
_S_PROJ = 66
_LAG = 28
_F1, _F2 = 64, 80


def _kernel(xa_hbm, ak, av, wqa, wota, xb_hbm, bk, bv, wqb, wotb, o_ref,
            kvbuf, xbuf, x8_scr, wqbuf, wobuf, q_scr, o_scr, z_scr, m_scr, l_scr, acc_scr, kv_sem, w_sem):
    PHA, PHB, CUTA, CUTB, STRIDE = _PH_A, _PH_B, _CUT_A, _CUT_B, _STRIDE
    S_W2, S_PROJ, LAG, F1, F2 = _S_W2, _S_PROJ, _LAG, _F1, _F2
    f32, bf16 = jnp.float32, jnp.bfloat16

    def in_order(once, fn):
        def body(_, c):
            fn()
            return c
        jax.lax.fori_loop(0, once, body, 0)

    def wait_region(ref, sem):
        pltpu.make_async_copy(ref, ref, sem).wait()

    def issue_kv(ksrc, vsrc, base, slot, ph):
        def pair(r, n, k_hi):
            g = pl.multiple_of(base + r, 8)
            kp, vp = (_HI, _LO) if k_hi else (_LO, _HI)
            pltpu.make_async_copy(ksrc.at[pl.ds(g, n)], kvbuf.at[slot, 0, pl.ds(r, n)],
                                  kv_sem.at[slot]).start(priority=kp)
            pltpu.make_async_copy(vsrc.at[pl.ds(g, n)], kvbuf.at[slot, 1, pl.ds(r, n)],
                                  kv_sem.at[slot]).start(priority=vp)

        off = ((_NB - 1) * (1 - STRIDE)) % _NB

        def block(j, k_hi):
            r0 = ph + ((STRIDE * j + off) % _NB) * 2 * _S

            def one(t, c):
                pair(pl.multiple_of(r0 + t * _S, 8), _S, k_hi)
                return c
            jax.lax.fori_loop(0, 2, one, 0)

        def two(jj, c):
            block(2 * jj, True)
            block(2 * jj + 1, False)
            return c

        pair(0, ph, False)
        jax.lax.fori_loop(0, _NB // 2 - 1, two, 0)
        block(_NB - 2, True)
        last = ph + (_NB - 1) * 2 * _S
        pair(last, _T - last, False)

    def issue_a(n):
        issue_kv(ak, av, n * _T, n % _NSLOT, PHA)

    def issue_b(n):
        issue_kv(bk, bv, (n - _NA) * _SK + (_SK - _W), n % _NSLOT, PHB)

    def issue_w(st0, st1, nslab, sig):
        def piece(st, j, c0, c1, prio):
            src, s0, dst, d0, _, sem = st
            r = pl.multiple_of((s0 + j) * 8, 8)
            d = pl.multiple_of((d0 + j) * 8, 8)
            pltpu.make_async_copy(src.at[pl.ds(r, 8), pl.ds(c0, c1 - c0)],
                                  dst.at[pl.ds(d, 8), pl.ds(c0, c1 - c0)], sem).start(priority=prio)

        def two(jj, c):
            once = jnp.minimum(jj + 1, 1)
            for k in range(2):
                j = (sig * (2 * jj + k)) % nslab
                nx = jnp.where(j + 1 == nslab, 0, j + 1)
                in_order(once, lambda: (piece(st0, j, st0[4], _HD, _HI), piece(st1, j, st1[4], _HD, _LO)))
                in_order(once, lambda: (piece(st0, nx, 0, st0[4], _HI), piece(st1, nx, 0, st1[4], _LO)))
            return c
        jax.lax.fori_loop(0, nslab // 2, two, 0)

    tail = [(0, 4, None, 3 * _NU, 4 * _NU), (8, 8, None, 4 * _NU, 5 * _NU)]
    for first, t, edges in ((24, 5, (0, 2048, _HD)), (40, 6, (0, 2048, 3072, _HD))):
        for c0, c1 in zip(edges[:-1], edges[1:]):
            tail.append((first, 8, (c0, c1), t * _NU + c0 // _UC, t * _NU + c1 // _UC))
    n_w = 4
    q_hi, q_lo = [], []
    for i, (first, n, cols, _, _) in enumerate(tail):
        for k in range(n + 1 if cols is None else n):
            for st in range(2):
                a = first + st * n
                if cols is None:
                    blk = ([(a + k - 1, CUTB, _HD)] if k > 0 else []) + ([(a + k, 0, CUTB)] if k < n else [])
                else:
                    blk = [(a + k,) + cols]
                (q_hi if (k + st) % 2 == 0 else q_lo).extend((i,) + p for p in blk)
    nh = len(q_hi) - LAG // 2
    lo_seq = q_lo[:nh] + [p for pr in zip(q_hi[nh:], q_lo[nh:]) for p in pr]
    fifo = [(p, _LO) for p in lo_seq[:LAG]]
    for i in range(nh):
        fifo += [(q_hi[i], _HI), (lo_seq[LAG + i], _LO)]
    assert len(fifo) == len(q_hi) + len(q_lo)

    def issue_tail(once, a, b):
        def start(entries):
            for (i, sl, c0, c1), prio in entries:
                pltpu.make_async_copy(wotb.at[pl.ds(sl * 8, 8), pl.ds(c0, c1 - c0)],
                                      wobuf.at[pl.ds(_D + sl * 8, 8), pl.ds(c0, c1 - c0)],
                                      w_sem.at[n_w + i]).start(priority=prio)
        for k in range(a, b, 2):
            in_order(once, functools.partial(start, fifo[k:min(k + 2, b)]))

    def wait_tail(i):
        first, n, cols, _, _ = tail[i]
        c0, c1 = cols or (0, _HD)
        wait_region(wobuf.at[pl.ds(_D + first * 8, 16 * n), pl.ds(c0, c1 - c0)], w_sem.at[n_w + i])

    xc = (pltpu.make_async_copy(xa_hbm, xbuf.at[0], w_sem.at[1]),
          pltpu.make_async_copy(xb_hbm, xbuf.at[1], w_sem.at[1]))
    for cp in xc:
        cp.start()
    half = _NSL // 2
    issue_w((wqa, 0, wqbuf.at[0], 0, CUTA, w_sem.at[0]), (wqa, half, wqbuf.at[0], half, CUTA, w_sem.at[0]),
            half, _SIG_1)

    def pre(n, c):
        issue_a(n)
        return c
    jax.lax.fori_loop(0, _LA, pre, 0)

    for ref in (o_scr, z_scr, m_scr, l_scr, acc_scr):
        ref[...] = jnp.zeros(ref.shape, f32)
    for cp in xc:
        cp.wait()
    rx = jax.lax.broadcasted_iota(jnp.int32, (8, _D), 0)
    xs = []
    for ab in range(2):
        x = xbuf[ab].astype(f32)
        xs.append(jnp.where(rx % 2 == 0, jnp.broadcast_to(x[0:1], (8, _D)), jnp.broadcast_to(x[1:2], (8, _D))))
    x8_scr[...] = jnp.where(rx < 4, xs[0], xs[1])
    wait_region(wqbuf.at[0], w_sem.at[0])

    row = jax.lax.broadcasted_iota(jnp.int32, (8, _DH), 0)
    lane = jax.lax.broadcasted_iota(jnp.int32, (8, 128), 1)

    def unit(u, c):
        t, cb = u // _NU, u % _NU
        per = _UC // _DH
        lhs = jnp.concatenate([o_scr[cb * per + i] for i in range(per)], axis=1).astype(bf16)
        w = wobuf[pl.ds(pl.multiple_of(t * 128, 128), 128), pl.ds(pl.multiple_of(cb * _UC, _UC), _UC)]
        z_scr[t] += jax.lax.dot_general(lhs, w, _NT, preferred_element_type=f32)
        return c

    def finish_tile(t):
        z = z_scr[t]
        s = z + pltpu.roll(z, 6, 0)
        if (t + 1) * 128 <= _D:
            w = s
        elif t * 128 >= _D:
            w = pltpu.roll(s, 4, 0)
        else:
            w = jnp.where(lane < _D - t * 128, s, pltpu.roll(s, 4, 0))
        o_ref[:, t * 128:(t + 1) * 128] = w[0:2].astype(o_ref.dtype)

    sched = [(S_PROJ + t, t * _NU, (t + 1) * _NU) for t in range(3)]
    sched += [(_NS + i, c[3], c[4]) for i, c in enumerate(tail)]
    first_of_last_tile = len(tail) - 3

    def event(s, carry):
        n = s + _LA
        once = jnp.minimum(s, 1)

        @pl.when(n < _NA)
        def _():
            issue_a(n)

        @pl.when(jnp.logical_and(n >= _NA, n < _NS))
        def _():
            issue_b(n)

        @pl.when(s == S_W2)
        def _():
            issue_w((wqb, 0, wqbuf.at[1], 0, CUTB, w_sem.at[2]), (wota, 0, wobuf, 0, CUTA, w_sem.at[3]),
                    _NSL, _SIG_2)

        @pl.when(n == _NS)
        def _():
            issue_tail(once, 0, F1)

        @pl.when(n == _NS + 1)
        def _():
            issue_tail(once, F1, F2)

        @pl.when(s == _NA)
        def _():
            wait_region(wqbuf.at[1], w_sem.at[2])
            wait_region(wobuf.at[pl.ds(0, _D)], w_sem.at[3])

        @pl.when(s < _NS)
        def _():
            is_a = s < _NA
            p = jnp.where(is_a, s // _NC, s - _NA)
            first = jnp.logical_or(jnp.logical_not(is_a), s % _NC == 0)
            last = jnp.logical_or(jnp.logical_not(is_a), s % _NC == _NC - 1)
            ab = jnp.where(is_a, 0, 1)
            b, h = p // _HKV, p % _HKV
            slot = s % _NSLOT

            @pl.when(jnp.logical_and(first, b == 0))
            def _():
                w = wqbuf[ab, :, pl.ds(pl.multiple_of(h * 2 * _DH, 2 * _DH), 2 * _DH)]
                qq = jnp.dot(x8_scr[...].astype(bf16), w, preferred_element_type=f32)
                qh = jnp.where((row // 2) % 2 == 0, qq[:, :_DH], qq[:, _DH:])
                q_scr[h] = qh.astype(bf16).astype(f32) * (_DH ** -0.5)

            q = q_scr[h].astype(bf16)
            wait_region(kvbuf.at[slot], kv_sem.at[slot])
            sc = jax.lax.dot_general(q, kvbuf[slot, 0], _NT, preferred_element_type=f32)
            m_old = jnp.where(first, -jnp.inf, m_scr[:, 0:1])
            l_old = jnp.where(first, 0.0, l_scr[:, 0:1])
            acc_old = jnp.where(first, 0.0, acc_scr[...])
            m_new = jnp.maximum(m_old, jnp.max(sc, axis=-1, keepdims=True))
            alpha = jnp.exp(m_old - m_new)
            pr = jnp.exp(sc - m_new)
            l_new = alpha * l_old + jnp.sum(pr, axis=-1, keepdims=True)
            acc_new = alpha * acc_old + jnp.dot(pr.astype(bf16), kvbuf[slot, 1], preferred_element_type=f32)
            m_scr[...] = jnp.broadcast_to(m_new, m_scr.shape)
            l_scr[...] = jnp.broadcast_to(l_new, l_scr.shape)
            acc_scr[...] = acc_new

            @pl.when(last)
            def _():
                o = acc_new / l_new
                for g in range(2):
                    o_scr[2 * h + g] = jnp.where(row == 4 * ab + 2 * g + b, o, o_scr[2 * h + g])

        @pl.when(s == _NS - 1)
        def _():
            issue_tail(once, F2, len(fifo))

        for i in range(len(tail)):
            @pl.when(s == _NS + i)
            def _():
                if i == first_of_last_tile:
                    for t in range(6):
                        finish_tile(t)
                wait_tail(i)

        lo = hi = jnp.int32(0)
        for e, a, z in sched:
            lo = jnp.where(s == e, a, lo)
            hi = jnp.where(s == e, z, hi)
        jax.lax.fori_loop(lo, hi, unit, 0)
        return carry

    jax.lax.fori_loop(0, _NS + len(tail), event, 0)
    finish_tile(6)


@jax.jit
def pallas_concat_heads__gqa_block_cached__sliding_block_cached__decode_kernel(
    A_x: jax.Array,
    A_k_cache: jax.Array,
    A_v_cache: jax.Array,
    A_wq: jax.Array,
    A_wo: jax.Array,
    B_x: jax.Array,
    B_k_cache: jax.Array,
    B_v_cache: jax.Array,
    B_wq: jax.Array,
    B_wo: jax.Array,
):
    bf16, f32 = jnp.bfloat16, jnp.float32
    flat = lambda t: t.reshape(_B * _HKV * _SK, _DH)
    extra = {}
    if hasattr(pltpu.CompilerParams(), "disable_semaphore_checks"):
        extra["disable_semaphore_checks"] = True
    out = pl.pallas_call(
        _kernel,
        in_specs=[pl.BlockSpec(memory_space=pl.ANY)] * 10,
        out_specs=pl.BlockSpec(memory_space=pltpu.VMEM),
        out_shape=jax.ShapeDtypeStruct((_B, 2 * _D), bf16),
        scratch_shapes=[
            pltpu.VMEM((_NSLOT, 2, _T, _DH), bf16),
            pltpu.VMEM((2, _B, _D), bf16),
            pltpu.VMEM((8, _D), f32),
            pltpu.VMEM((2, _D, _HD), bf16),
            pltpu.VMEM((2 * _D, _HD), bf16),
            pltpu.VMEM((_HKV, 8, _DH), f32),
            pltpu.VMEM((_HQ, 8, _DH), f32),
            pltpu.VMEM((7, 8, 128), f32),
            pltpu.VMEM((8, 128), f32),
            pltpu.VMEM((8, 128), f32),
            pltpu.VMEM((8, _DH), f32),
            pltpu.SemaphoreType.DMA((_NSLOT,)),
            pltpu.SemaphoreType.DMA((11,)),
        ],
        compiler_params=pltpu.CompilerParams(vmem_limit_bytes=64 * 1024 * 1024, **extra),
    )(A_x.reshape(_B, _D), flat(A_k_cache), flat(A_v_cache), A_wq, A_wo.T,
      B_x.reshape(_B, _D), flat(B_k_cache), flat(B_v_cache), B_wq, B_wo.T)
    return out.reshape(_B, 1, 2 * _D)
```
